```python
import jax
import jax.numpy as jnp

def _softmax(x, axis=-1):
    return jax.nn.softmax(x, axis=axis)

def _gelu(x):
    return jax.nn.gelu(x, approximate=True)

def _silu(x):
    return jax.nn.silu(x)

def _sigmoid(x):
    return jax.nn.sigmoid(x)

def _layernorm(x, axis=-1, eps=1e-05):
    m = jnp.mean(x, axis=axis, keepdims=True)
    v = jnp.var(x, axis=axis, keepdims=True)
    return (x - m) / jnp.sqrt(v + eps)

def _scatter_add(tgt, idx, src, axis=0):
    return tgt.at[idx].add(src)

def _segment_sum(src, seg, n):
    return jax.ops.segment_sum(src, seg, n)

class _Rng:

    def __init__(self, key):
        self._k = key

    def _next(self):
        self._k, sub = jax.random.split(self._k)
        return sub

    def normal(self, shape):
        return jax.random.normal(self._next(), shape, dtype=jnp.bfloat16)

    def randint(self, lo, hi, shape):
        return jax.random.randint(self._next(), shape, lo, hi, dtype=jnp.int32)

    def uniform(self, shape, lo=0.0, hi=1.0):
        return jax.random.uniform(self._next(), shape, jnp.bfloat16, lo, hi)

    def permutation(self, n):
        return jax.random.permutation(self._next(), n)
kernel_name = 'adaLN_cond__sliding_block_cached__mixer_channel_mlp__decode'

def setup_inputs():
    _rng = _Rng(jax.random.key(int.from_bytes(__import__("os").urandom(4), "little")))
    _w = lambda a: (lambda t: t.astype(jnp.bfloat16) if jnp.issubdtype(t.dtype, jnp.floating) else t)(jnp.asarray(a))

    def _A_setup():
        B, Sq, D = (8, 1, 640)
        Hq, Hkv, Sk, Dh = (32, 32, 4096, 192)
        assert Hq % Hkv == 0, (Hq, Hkv)
        return {'x': _w((lambda *s: _rng.normal(s) * 0.05)(B, Sq, D)), 'k_cache': _w((lambda *s: _rng.normal(s) * 0.05)(B, Hkv, Sk, Dh)), 'v_cache': _w((lambda *s: _rng.normal(s) * 0.05)(B, Hkv, Sk, Dh)), 'wq': _w((lambda *s: _rng.normal(s) * 0.05)(D, Hq * Dh) * D ** (-0.5)), 'wo': _w((lambda *s: _rng.normal(s) * 0.05)(Hq * Dh, D) * (Hq * Dh) ** (-0.5))}
    _A_in = _A_setup()

    def _B_setup():
        B, S, D, F = (8, 1, 640, 1536)
        return {'x': _w((lambda *s: _rng.normal(s) * 0.05)(B, S, D)), 'w1': _w((lambda *s: _rng.normal(s) * 0.05)(D, F) * D ** (-0.5)), 'b1': _w((lambda *s: _rng.normal(s) * 0.05)(F)), 'w2': _w((lambda *s: _rng.normal(s) * 0.05)(F, D) * F ** (-0.5)), 'b2': _w((lambda *s: _rng.normal(s) * 0.05)(D))}
    _B_in = _B_setup()
    return {'A_x': _A_in['x'], 'A_k_cache': _A_in['k_cache'], 'A_v_cache': _A_in['v_cache'], 'A_wq': _A_in['wq'], 'A_wo': _A_in['wo'], 'B_x': _B_in['x'], 'B_w1': _B_in['w1'], 'B_b1': _B_in['b1'], 'B_w2': _B_in['w2'], 'B_b2': _B_in['b2'], 'c': _w((lambda *s: _rng.normal(s) * 0.05)(8, 640)), 'w_mod': _w((lambda *s: _rng.normal(s) * 0.05)(640, 6 * 640) * 640 ** (-0.5))}

def reference(A_x, A_k_cache, A_v_cache, A_wq, A_wo, B_x, B_w1, B_b1, B_w2, B_b2, c, w_mod):

    def _A_ref(x, k_cache, v_cache, wq, wo):
        B, Sq, D = x.shape
        Hq, Dh = (32, 192)
        Hkv, Sk = (k_cache.shape[1], k_cache.shape[2])
        W = min(4096, max(256, Sk // 4))
        rep = Hq // Hkv
        q = (lambda x, *d: x.transpose(*d))((x @ wq).reshape(B, Sq, Hq, Dh), 0, 2, 1, 3)
        k = jnp.repeat(k_cache[:, :, Sk - W:, :], rep, axis=1)
        v = jnp.repeat(v_cache[:, :, Sk - W:, :], rep, axis=1)
        scores = jnp.einsum('bhqd,bhkd->bhqk', q, k) * Dh ** (-0.5)
        p = _softmax(scores, axis=-1)
        o = jnp.einsum('bhqk,bhkd->bhqd', p, v)
        return (lambda x, *d: x.transpose(*d))(o, 0, 2, 1, 3).reshape(B, Sq, Hq * Dh) @ wo

    def _B_ref(x, w1, b1, w2, b2):
        y = _layernorm(x, axis=-1)
        h = _gelu(jnp.einsum('bsd,df->bsf', y, w1) + b1)
        return jnp.einsum('bsf,fd->bsd', h, w2) + b2
    x = A_x
    mod = (_silu(c) @ w_mod).reshape(c.shape[0], 6, 1, -1)
    sa, ca, ga, sb, cb, gb = (mod[:, 0].copy(), mod[:, 1].copy(), mod[:, 2].copy(), mod[:, 3].copy(), mod[:, 4].copy(), mod[:, 5].copy())
    h = _layernorm(x, axis=-1) * (1 + ca) + sa
    x = x + ga * _A_ref(h, A_k_cache, A_v_cache, A_wq, A_wo)
    h = _layernorm(x, axis=-1) * (1 + cb) + sb
    x = x + gb * _B_ref(h, B_w1, B_b1, B_w2, B_b2)
    return x
```

```python
import jax
import jax.numpy as jnp
from jax import lax
import jax.experimental.pallas as pl
import jax.experimental.pallas.tpu as pltpu

F32 = jnp.float32
BF16 = jnp.bfloat16

G = 8
NBUF = 4


def _layernorm(x, eps=1e-5):
    m = jnp.mean(x, axis=-1, keepdims=True)
    d = x - m
    v = jnp.mean(d * d, axis=-1, keepdims=True)
    return d * lax.rsqrt(v + eps)


@jax.jit
def pallas_adaLN_cond__sliding_block_cached__mixer_channel_mlp__decode_kernel(
    A_x: jax.Array,
    A_k_cache: jax.Array,
    A_v_cache: jax.Array,
    A_wq: jax.Array,
    A_wo: jax.Array,
    B_x: jax.Array,
    B_w1: jax.Array,
    B_b1: jax.Array,
    B_w2: jax.Array,
    B_b2: jax.Array,
    c: jax.Array,
    w_mod: jax.Array,
):
    del B_x
    B, Sq, D = A_x.shape
    _, H, Sk, Dh = A_k_cache.shape
    F = B_w1.shape[1]
    W = min(4096, max(256, Sk // 4))
    R = G * Dh
    NG = H // G
    NCH = B * NG
    scale = Dh ** (-0.5)

    def kern(x_hbm, k_hbm, v_hbm, wq_hbm, wo_hbm, w1_hbm, b1_hbm, w2_hbm, b2_hbm, c_hbm, wm_hbm,
             o_ref,
             x_v, c_v, b1_v, b2_v, wma_v, wmb_v, wq_v, wo_v, w1_v, w2_v, kb, vb, q_s, a_s,
             sem_w, sem_k, sem_v):
        def kcp(i, slot):
            return pltpu.make_async_copy(
                k_hbm.at[pl.ds(i * R, R), pl.ds(Sk - W, W)], kb.at[slot], sem_k.at[slot])

        def vcp(i, slot):
            return pltpu.make_async_copy(
                v_hbm.at[pl.ds(i * R, R), pl.ds(Sk - W, W)], vb.at[slot], sem_v.at[slot])

        cp_c = pltpu.make_async_copy(c_hbm, c_v, sem_w.at[0])
        cp_x = pltpu.make_async_copy(x_hbm, x_v, sem_w.at[1])
        cp_wma = pltpu.make_async_copy(wm_hbm.at[:, pl.ds(0, 2 * D)], wma_v, sem_w.at[2])
        cp_wq = pltpu.make_async_copy(wq_hbm, wq_v, sem_w.at[3])
        cp_wo = pltpu.make_async_copy(wo_hbm, wo_v, sem_w.at[4])
        cp_wmb = pltpu.make_async_copy(wm_hbm.at[:, pl.ds(2 * D, 4 * D)], wmb_v, sem_w.at[5])
        cp_b1 = pltpu.make_async_copy(b1_hbm, b1_v, sem_w.at[6])
        cp_b2 = pltpu.make_async_copy(b2_hbm, b2_v, sem_w.at[7])
        cp_w1 = pltpu.make_async_copy(w1_hbm, w1_v, sem_w.at[8])
        cp_w2 = pltpu.make_async_copy(w2_hbm, w2_v, sem_w.at[9])

        cp_wma.start()
        cp_c.start()
        cp_x.start()
        cp_wq.start()
        for i in range(NBUF):
            kcp(i, i).start()
            vcp(i, i).start()
        cp_b1.start()
        cp_b2.start()

        cp_c.wait()
        cp_x.wait()
        cp_wma.wait()
        cf = c_v[...].astype(F32)
        sc = (cf * jax.nn.sigmoid(cf)).astype(BF16)
        moda = jnp.dot(sc, wma_v[...], preferred_element_type=F32)
        x = x_v[...].astype(F32)
        h = _layernorm(x) * (1.0 + moda[:, D:]) + moda[:, :D]
        cp_wq.wait()
        q_s[...] = jnp.dot(h.astype(BF16), wq_v[...], preferred_element_type=F32) * scale

        row = lax.broadcasted_iota(jnp.int32, (G, R), 0)
        col = lax.broadcasted_iota(jnp.int32, (G, R), 1)
        diag = (col >= row * Dh) & (col < (row + 1) * Dh)

        def body(i, _):
            slot = i % NBUF
            b = i // NG
            g = i % NG
            off = pl.multiple_of(g * R, 128)
            qrow = q_s[pl.ds(b, 1), pl.ds(off, R)]
            qbd = jnp.where(diag, jnp.broadcast_to(qrow, (G, R)), 0.0).astype(BF16)
            kcp(i, slot).wait()
            s = jnp.dot(qbd, kb[slot], preferred_element_type=F32)

            @pl.when(i + NBUF < NCH)
            def _():
                kcp(i + NBUF, slot).start()

            m = jnp.max(s, axis=-1, keepdims=True)
            e = jnp.exp(s - m)
            l = jnp.sum(e, axis=-1, keepdims=True)
            p = (e / l).astype(BF16)
            vcp(i, slot).wait()
            o = lax.dot_general(p, vb[slot], (((1,), (1,)), ((), ())), preferred_element_type=F32)

            @pl.when(i + NBUF < NCH)
            def _():
                vcp(i + NBUF, slot).start()

            @pl.when(i + NBUF == NCH - 1)
            def _():
                cp_wo.start()
                cp_wmb.start()
                cp_w1.start()
                cp_w2.start()

            a_s[pl.ds(b, 1), pl.ds(off, R)] = jnp.sum(jnp.where(diag, o, 0.0), axis=0, keepdims=True)

        lax.fori_loop(0, NCH, body, None)

        cp_wo.wait()
        attn = jnp.dot(a_s[...].astype(BF16), wo_v[...], preferred_element_type=F32)
        cp_wmb.wait()
        modb = jnp.dot(sc, wmb_v[...], preferred_element_type=F32)
        ga, sb, cb, gb = (modb[:, j * D:(j + 1) * D] for j in range(4))
        x1 = x + ga * attn
        h2 = _layernorm(x1) * (1.0 + cb) + sb
        y = _layernorm(h2)
        cp_b1.wait()
        cp_b2.wait()
        cp_w1.wait()
        b1r = b1_v[...].astype(F32).reshape(1, F)
        b2r = b2_v[...].astype(F32).reshape(1, D)
        u = jnp.dot(y.astype(BF16), w1_v[...], preferred_element_type=F32) + b1r
        gl = jax.nn.gelu(u, approximate=True)
        cp_w2.wait()
        z = jnp.dot(gl.astype(BF16), w2_v[...], preferred_element_type=F32) + b2r
        o_ref[...] = (x1 + gb * z).astype(o_ref.dtype)

    kt = jnp.swapaxes(A_k_cache, 2, 3).reshape(B * H * Dh, Sk)
    vt = jnp.swapaxes(A_v_cache, 2, 3).reshape(B * H * Dh, Sk)
    anyspec = pl.BlockSpec(memory_space=pl.ANY)
    out = pl.pallas_call(
        kern,
        out_shape=jax.ShapeDtypeStruct((B, D), A_x.dtype),
        in_specs=[anyspec] * 11,
        scratch_shapes=[
            pltpu.VMEM((B, D), BF16), pltpu.VMEM((B, D), BF16),
            pltpu.VMEM((F,), BF16), pltpu.VMEM((D,), BF16),
            pltpu.VMEM((D, 2 * D), BF16), pltpu.VMEM((D, 4 * D), BF16),
            pltpu.VMEM((D, H * Dh), BF16), pltpu.VMEM((H * Dh, D), BF16),
            pltpu.VMEM((D, F), BF16), pltpu.VMEM((F, D), BF16),
            pltpu.VMEM((NBUF, R, W), BF16), pltpu.VMEM((NBUF, R, W), BF16),
            pltpu.VMEM((B, H * Dh), F32), pltpu.VMEM((B, H * Dh), F32),
            pltpu.SemaphoreType.DMA((10,)),
            pltpu.SemaphoreType.DMA((NBUF,)),
            pltpu.SemaphoreType.DMA((NBUF,)),
        ],
        compiler_params=pltpu.CompilerParams(vmem_limit_bytes=100 * 2**20),
    )(A_x.reshape(B, D), kt, vt, A_wq, A_wo, B_w1, B_b1, B_w2, B_b2, c, w_mod)
    return out.reshape(B, Sq, D)
```

```python
import jax
import jax.numpy as jnp
from jax import lax
import jax.experimental.pallas as pl
import jax.experimental.pallas.tpu as pltpu

F32 = jnp.float32
BF16 = jnp.bfloat16

HEADS_PER_CHUNK = 8
NUM_SLOTS = 2
W2_SPLIT = (4, 4, 3, 1)


def _layernorm(x, eps=1e-5):
    m = jnp.mean(x, axis=-1, keepdims=True)
    d = x - m
    v = jnp.mean(d * d, axis=-1, keepdims=True)
    return d * lax.rsqrt(v + eps)


def _dot(a, b):
    return jnp.dot(a, b, preferred_element_type=F32)


@jax.jit
def pallas_adaLN_cond__sliding_block_cached__mixer_channel_mlp__decode_kernel(
    A_x: jax.Array,
    A_k_cache: jax.Array,
    A_v_cache: jax.Array,
    A_wq: jax.Array,
    A_wo: jax.Array,
    B_x: jax.Array,
    B_w1: jax.Array,
    B_b1: jax.Array,
    B_w2: jax.Array,
    B_b2: jax.Array,
    c: jax.Array,
    w_mod: jax.Array,
):
    del B_x
    B, Sq, D = A_x.shape
    _, H, Sk, Dh = A_k_cache.shape
    F = B_w1.shape[1]
    W = min(4096, max(256, Sk // 4))
    G = HEADS_PER_CHUNK
    R = G * Dh
    NG = H // G
    NCH = B * NG
    scale = Dh ** (-0.5)
    assert Sq == 1 and H % G == 0 and R % 128 == 0 and A_wq.shape[1] == H * Dh
    assert NCH >= NUM_SLOTS and F % (128 * sum(W2_SPLIT)) == 0
    w2_rows = [F // sum(W2_SPLIT) * n for n in W2_SPLIT]
    w2_offs = [sum(w2_rows[:j]) for j in range(len(w2_rows))]

    def kernel(x_hbm, k_hbm, v_hbm, wq_hbm, wo_hbm, w1_hbm, b1_hbm, w2_hbm, b2_hbm, c_hbm,
               wm_hbm, o_ref,
               x_v, c_v, b1_v, b2_v, wma_v, wmb_v, wq_v, wo_v, w1_v, w2_v, kv_v, q_v, att_v,
               sem_w, sem_kv):

        def start_kv(i, slot):
            for h in range(G):
                src = (pl.ds(i * R + h * Dh, Dh), pl.ds(Sk - W, W))
                dst = pl.ds(h * Dh, Dh)
                pltpu.make_async_copy(k_hbm.at[src], kv_v.at[slot, 0, dst], sem_kv.at[slot]).start()
                pltpu.make_async_copy(v_hbm.at[src], kv_v.at[slot, 1, dst], sem_kv.at[slot]).start()

        def wait_kv(slot):
            pltpu.make_async_copy(kv_v.at[slot], kv_v.at[slot], sem_kv.at[slot]).wait()

        cp_first = [
            pltpu.make_async_copy(wm_hbm.at[:, pl.ds(0, 2 * D)], wma_v, sem_w.at[0]),
            pltpu.make_async_copy(c_hbm, c_v, sem_w.at[0]),
            pltpu.make_async_copy(x_hbm, x_v, sem_w.at[0]),
            pltpu.make_async_copy(b1_hbm, b1_v, sem_w.at[0]),
            pltpu.make_async_copy(b2_hbm, b2_v, sem_w.at[0]),
        ]
        cp_wq = pltpu.make_async_copy(wq_hbm, wq_v, sem_w.at[1])
        cp_wo = pltpu.make_async_copy(wo_hbm, wo_v, sem_w.at[0])
        cp_wmb = pltpu.make_async_copy(wm_hbm.at[:, pl.ds(2 * D, 4 * D)], wmb_v, sem_w.at[1])
        cp_w1 = pltpu.make_async_copy(w1_hbm, w1_v, sem_w.at[2])
        cp_w2 = [
            pltpu.make_async_copy(w2_hbm.at[pl.ds(o, n)], w2_v.at[pl.ds(o, n)], sem_kv.at[j])
            for j, (o, n) in enumerate(zip(w2_offs, w2_rows))
        ]

        for cp in cp_first:
            cp.start()
        cp_wq.start()
        for cp in cp_first:
            cp.wait()
        for i in range(NUM_SLOTS):
            start_kv(i, i)

        cf = c_v[...].astype(F32)
        silu_c = (cf * jax.nn.sigmoid(cf)).astype(BF16)
        mod_a = _dot(silu_c, wma_v[...])
        sa, ca = mod_a[:, :D], mod_a[:, D:]
        x = x_v[...].astype(F32)
        h = _layernorm(x) * (1.0 + ca) + sa
        cp_wq.wait()
        q_v[...] = _dot(h.astype(BF16), wq_v[...]) * scale

        row = lax.broadcasted_iota(jnp.int32, (G, R), 0)
        col = lax.broadcasted_iota(jnp.int32, (G, R), 1)
        diag = (col >= row * Dh) & (col < (row + 1) * Dh)

        def attend(i, carry):
            slot = i % NUM_SLOTS
            b = pl.ds(i // NG, 1)
            heads = pl.ds(pl.multiple_of((i % NG) * R, 128), R)
            q = jnp.where(diag, jnp.broadcast_to(q_v[b, heads], (G, R)), 0.0).astype(BF16)
            wait_kv(slot)

            @pl.when(i + NUM_SLOTS == NCH)
            def _():
                cp_wo.start()
                cp_wmb.start()
                cp_w1.start()

            s = _dot(q, kv_v[slot, 0])
            e = jnp.exp(s - jnp.max(s, axis=-1, keepdims=True))
            p = (e / jnp.sum(e, axis=-1, keepdims=True)).astype(BF16)
            o = lax.dot_general(p, kv_v[slot, 1], (((1,), (1,)), ((), ())),
                                preferred_element_type=F32)
            att_v[b, heads] = jnp.sum(jnp.where(diag, o, 0.0), axis=0, keepdims=True)

            @pl.when(i + NUM_SLOTS < NCH)
            def _():
                start_kv(i + NUM_SLOTS, slot)

            return carry

        lax.fori_loop(0, NCH, attend, None)

        for cp in cp_w2:
            cp.start()
        cp_wo.wait()
        attn = _dot(att_v[...].astype(BF16), wo_v[...])
        cp_wmb.wait()
        mod_b = _dot(silu_c, wmb_v[...])
        ga, sb, cb, gb = (mod_b[:, j * D:(j + 1) * D] for j in range(4))
        x = x + ga * attn
        y = _layernorm(_layernorm(x) * (1.0 + cb) + sb)
        b1 = b1_v[...].astype(F32).reshape(1, F)
        b2 = b2_v[...].astype(F32).reshape(1, D)
        cp_w1.wait()
        u = jax.nn.gelu(_dot(y.astype(BF16), w1_v[...]) + b1, approximate=True).astype(BF16)
        z = jnp.broadcast_to(b2, (B, D))
        for cp, o, n in zip(cp_w2, w2_offs, w2_rows):
            cp.wait()
            z = z + _dot(u[:, o:o + n], w2_v[pl.ds(o, n), :])
        o_ref[...] = (x + gb * z).astype(o_ref.dtype)

    kt = jnp.swapaxes(A_k_cache, 2, 3).reshape(B * H * Dh, Sk)
    vt = jnp.swapaxes(A_v_cache, 2, 3).reshape(B * H * Dh, Sk)
    out = pl.pallas_call(
        kernel,
        out_shape=jax.ShapeDtypeStruct((B, D), A_x.dtype),
        in_specs=[pl.BlockSpec(memory_space=pl.ANY)] * 11,
        scratch_shapes=[
            pltpu.VMEM((B, D), A_x.dtype),
            pltpu.VMEM((B, D), c.dtype),
            pltpu.VMEM((F,), B_b1.dtype),
            pltpu.VMEM((D,), B_b2.dtype),
            pltpu.VMEM((D, 2 * D), w_mod.dtype),
            pltpu.VMEM((D, 4 * D), w_mod.dtype),
            pltpu.VMEM((D, H * Dh), A_wq.dtype),
            pltpu.VMEM((H * Dh, D), A_wo.dtype),
            pltpu.VMEM((D, F), B_w1.dtype),
            pltpu.VMEM((F, D), B_w2.dtype),
            pltpu.VMEM((NUM_SLOTS, 2, R, W), A_k_cache.dtype),
            pltpu.VMEM((B, H * Dh), F32),
            pltpu.VMEM((B, H * Dh), F32),
            pltpu.SemaphoreType.DMA((3,)),
            pltpu.SemaphoreType.DMA((max(NUM_SLOTS, len(W2_SPLIT)),)),
        ],
        compiler_params=pltpu.CompilerParams(vmem_limit_bytes=100 * 2**20),
    )(A_x.reshape(B, D), kt, vt, A_wq, A_wo, B_w1, B_b1, B_w2, B_b2, c, w_mod)
    return out.reshape(B, Sq, D)
```

```python
import jax
import jax.numpy as jnp
from jax import lax
import jax.experimental.pallas as pl
import jax.experimental.pallas.tpu as pltpu

F32 = jnp.float32
BF16 = jnp.bfloat16

HEADS_PER_CHUNK = 8
NUM_SLOTS = 2
W2_SPLIT = (8, 3, 1)


def _layernorm(x, eps=1e-5):
    m = jnp.mean(x, axis=-1, keepdims=True)
    d = x - m
    v = jnp.mean(d * d, axis=-1, keepdims=True)
    return d * lax.rsqrt(v + eps)


def _dot(a, b):
    return jnp.dot(a, b, preferred_element_type=F32)


@jax.jit
def pallas_adaLN_cond__sliding_block_cached__mixer_channel_mlp__decode_kernel(
    A_x: jax.Array,
    A_k_cache: jax.Array,
    A_v_cache: jax.Array,
    A_wq: jax.Array,
    A_wo: jax.Array,
    B_x: jax.Array,
    B_w1: jax.Array,
    B_b1: jax.Array,
    B_w2: jax.Array,
    B_b2: jax.Array,
    c: jax.Array,
    w_mod: jax.Array,
):
    del B_x
    B, Sq, D = A_x.shape
    _, H, Sk, Dh = A_k_cache.shape
    F = B_w1.shape[1]
    W = min(4096, max(256, Sk // 4))
    G = HEADS_PER_CHUNK
    R = G * Dh
    NG = H // G
    NCH = B * NG
    scale = Dh ** (-0.5)
    assert Sq == 1 and H % G == 0 and R % 128 == 0 and A_wq.shape[1] == H * Dh
    assert NCH >= NUM_SLOTS and F % (128 * sum(W2_SPLIT)) == 0
    w2_rows = [F // sum(W2_SPLIT) * n for n in W2_SPLIT]
    w2_offs = [sum(w2_rows[:j]) for j in range(len(w2_rows))]

    def kernel(x_hbm, k_hbm, v_hbm, wq_hbm, wo_hbm, w1_hbm, b1_hbm, w2_hbm, b2_hbm, c_hbm,
               wm_hbm, o_ref,
               x_v, c_v, b1_v, b2_v, wm_v, wq_v, wo_v, w1_v, w2_v, kv_v, q_v, att_v,
               sem_w, sem_kv):

        def start_kv(i, slot):
            for h in range(G):
                src = (pl.ds(i * R + h * Dh, Dh), pl.ds(Sk - W, W))
                dst = pl.ds(h * Dh, Dh)
                pltpu.make_async_copy(k_hbm.at[src], kv_v.at[slot, 0, dst], sem_kv.at[slot]).start()
                pltpu.make_async_copy(v_hbm.at[src], kv_v.at[slot, 1, dst], sem_kv.at[slot]).start()

        def wait_kv(slot):
            pltpu.make_async_copy(kv_v.at[slot], kv_v.at[slot], sem_kv.at[slot]).wait()

        cp_first = [
            pltpu.make_async_copy(wm_hbm, wm_v, sem_w.at[0]),
            pltpu.make_async_copy(c_hbm, c_v, sem_w.at[0]),
            pltpu.make_async_copy(x_hbm, x_v, sem_w.at[0]),
            pltpu.make_async_copy(b1_hbm, b1_v, sem_w.at[0]),
            pltpu.make_async_copy(b2_hbm, b2_v, sem_w.at[0]),
        ]
        cp_wq = pltpu.make_async_copy(wq_hbm, wq_v, sem_w.at[1])
        cp_wo = pltpu.make_async_copy(wo_hbm, wo_v, sem_w.at[0])
        cp_w1 = pltpu.make_async_copy(w1_hbm, w1_v, sem_w.at[1])
        cp_w2 = [
            pltpu.make_async_copy(w2_hbm.at[pl.ds(o, n)], w2_v.at[pl.ds(o, n)], sem_kv.at[j])
            for j, (o, n) in enumerate(zip(w2_offs, w2_rows))
        ]

        for cp in cp_first:
            cp.start()
        cp_wq.start()
        for cp in cp_first:
            cp.wait()
        for i in range(NUM_SLOTS):
            start_kv(i, i)

        cf = c_v[...].astype(F32)
        silu_c = (cf * jax.nn.sigmoid(cf)).astype(BF16)
        mod = _dot(silu_c, wm_v[...])
        sa, ca, ga, sb, cb, gb = (mod[:, j * D:(j + 1) * D] for j in range(6))
        x = x_v[...].astype(F32)
        h = _layernorm(x) * (1.0 + ca) + sa
        cp_wq.wait()
        q_v[...] = _dot(h.astype(BF16), wq_v[...]) * scale

        row = lax.broadcasted_iota(jnp.int32, (G, R), 0)
        col = lax.broadcasted_iota(jnp.int32, (G, R), 1)
        diag = (col >= row * Dh) & (col < (row + 1) * Dh)

        def attend(i, carry):
            slot = i % NUM_SLOTS
            b = pl.ds(i // NG, 1)
            heads = pl.ds(pl.multiple_of((i % NG) * R, 128), R)
            q = jnp.where(diag, jnp.broadcast_to(q_v[b, heads], (G, R)), 0.0).astype(BF16)
            wait_kv(slot)

            @pl.when(i + NUM_SLOTS == NCH)
            def _():
                cp_wo.start()
                cp_w1.start()

            s = _dot(q, kv_v[slot, 0])
            e = jnp.exp(s - jnp.max(s, axis=-1, keepdims=True))
            p = (e / jnp.sum(e, axis=-1, keepdims=True)).astype(BF16)
            o = lax.dot_general(p, kv_v[slot, 1], (((1,), (1,)), ((), ())),
                                preferred_element_type=F32)
            att_v[b, heads] = jnp.sum(jnp.where(diag, o, 0.0), axis=0, keepdims=True)

            @pl.when(i + NUM_SLOTS < NCH)
            def _():
                start_kv(i + NUM_SLOTS, slot)

            return carry

        lax.fori_loop(0, NCH, attend, None)

        for cp in cp_w2:
            cp.start()
        cp_wo.wait()
        attn = _dot(att_v[...].astype(BF16), wo_v[...])
        x = x + ga * attn
        y = _layernorm(_layernorm(x) * (1.0 + cb) + sb)
        b1 = b1_v[...].astype(F32).reshape(1, F)
        b2 = b2_v[...].astype(F32).reshape(1, D)
        cp_w1.wait()
        u = jax.nn.gelu(_dot(y.astype(BF16), w1_v[...]) + b1, approximate=True).astype(BF16)
        z = jnp.broadcast_to(b2, (B, D))
        for cp, o, n in zip(cp_w2, w2_offs, w2_rows):
            cp.wait()
            z = z + _dot(u[:, o:o + n], w2_v[pl.ds(o, n), :])
        o_ref[...] = (x + gb * z).astype(o_ref.dtype)

    kt = jnp.swapaxes(A_k_cache, 2, 3).reshape(B * H * Dh, Sk)
    vt = jnp.swapaxes(A_v_cache, 2, 3).reshape(B * H * Dh, Sk)
    out = pl.pallas_call(
        kernel,
        out_shape=jax.ShapeDtypeStruct((B, D), A_x.dtype),
        in_specs=[pl.BlockSpec(memory_space=pl.ANY)] * 11,
        scratch_shapes=[
            pltpu.VMEM((B, D), A_x.dtype),
            pltpu.VMEM((B, D), c.dtype),
            pltpu.VMEM((F,), B_b1.dtype),
            pltpu.VMEM((D,), B_b2.dtype),
            pltpu.VMEM((D, 6 * D), w_mod.dtype),
            pltpu.VMEM((D, H * Dh), A_wq.dtype),
            pltpu.VMEM((H * Dh, D), A_wo.dtype),
            pltpu.VMEM((D, F), B_w1.dtype),
            pltpu.VMEM((F, D), B_w2.dtype),
            pltpu.VMEM((NUM_SLOTS, 2, R, W), A_k_cache.dtype),
            pltpu.VMEM((B, H * Dh), F32),
            pltpu.VMEM((B, H * Dh), F32),
            pltpu.SemaphoreType.DMA((2,)),
            pltpu.SemaphoreType.DMA((max(NUM_SLOTS, len(W2_SPLIT)),)),
        ],
        compiler_params=pltpu.CompilerParams(vmem_limit_bytes=100 * 2**20),
    )(A_x.reshape(B, D), kt, vt, A_wq, A_wo, B_w1, B_b1, B_w2, B_b2, c, w_mod)
    return out.reshape(B, Sq, D)
```
